```python
import jax
import jax.numpy as jnp

def _softmax(x, axis=-1):
    return jax.nn.softmax(x, axis=axis)

def _gelu(x):
    return jax.nn.gelu(x, approximate=True)

def _silu(x):
    return jax.nn.silu(x)

def _sigmoid(x):
    return jax.nn.sigmoid(x)

def _layernorm(x, axis=-1, eps=1e-05):
    m = jnp.mean(x, axis=axis, keepdims=True)
    v = jnp.var(x, axis=axis, keepdims=True)
    return (x - m) / jnp.sqrt(v + eps)

def _scatter_add(tgt, idx, src, axis=0):
    return tgt.at[idx].add(src)

def _segment_sum(src, seg, n):
    return jax.ops.segment_sum(src, seg, n)

class _Rng:

    def __init__(self, key):
        self._k = key

    def _next(self):
        self._k, sub = jax.random.split(self._k)
        return sub

    def normal(self, shape):
        return jax.random.normal(self._next(), shape, dtype=jnp.bfloat16)

    def randint(self, lo, hi, shape):
        return jax.random.randint(self._next(), shape, lo, hi, dtype=jnp.int32)

    def uniform(self, shape, lo=0.0, hi=1.0):
        return jax.random.uniform(self._next(), shape, jnp.bfloat16, lo, hi)

    def permutation(self, n):
        return jax.random.permutation(self._next(), n)
kernel_name = 'standalone__conformer_conv_module__speech'

def setup_inputs():
    _rng = _Rng(jax.random.key(int.from_bytes(__import__("os").urandom(4), "little")))
    _w = lambda a: (lambda t: t.astype(jnp.bfloat16) if jnp.issubdtype(t.dtype, jnp.floating) else t)(jnp.asarray(a))
    B, T, D, K = (2, 16000, 256, 31)
    return {'x': _w((lambda *s: _rng.normal(s) * 0.05)(B, T, D)), 'w_pw1': _w((lambda *s: _rng.normal(s) * 0.05)(D, 2 * D)), 'dw': _w((lambda *s: _rng.normal(s) * 0.05)(K, D)), 'w_pw2': _w((lambda *s: _rng.normal(s) * 0.05)(D, D))}

def reference(x, w_pw1, dw, w_pw2):
    B, T, D = x.shape
    K = dw.shape[0]
    h = x @ w_pw1
    a, b = (h[..., :D].copy(), h[..., D:].copy())
    h = a * _sigmoid(b)
    pad = K // 2
    hp = jnp.pad(h, ((0, 0), (pad, pad), (0, 0)))
    out = jnp.zeros_like(h)
    for i in range(K):
        out = out + hp[:, i:i + T, :] * dw[i][None, None, :]
    return _silu(out) @ w_pw2
```

```python
import functools, itertools, jax, jax.numpy as jnp
import jax.experimental.pallas as pl
import jax.experimental.pallas.tpu as pltpu

F32 = jnp.float32
BF = jnp.bfloat16
S = 8
LV = 3
P = 32


@jax.jit
def pallas_standalone__conformer_conv_module__speech_kernel(x, w_pw1, dw, w_pw2):
    NP, HS, ZS, MS, od, pp, R, flags = 5, 33, 17, 1, 2, 54, 2, None
    grp = [(j,) for j in range(NP)]
    B, T, D = x.shape
    K = dw.shape[0]
    Q = S // B
    L = T // Q
    TB = NP * P
    NS = L // TB
    RING = TB // 8
    NH = D // 128
    paths = list(itertools.product(range(3), repeat=LV))
    pid = {p: i for i, p in enumerate(paths)}

    def kern(x_ref, xl_ref, xf_ref, w1_ref, dw_ref, w2_ref, o_ref, w1s, w2s, wt, hb, sb, zb):
        i = pl.program_id(0)

        def weights():
            for c in range(NH):
                w = jnp.concatenate([w1_ref[:, (e * NH + c) * 128:(e * NH + c + 1) * 128] for e in range(2)], 1)
                w1s[c] = pltpu.bitcast((w.astype(F32) * 0.5).astype(BF), jnp.uint32)
            w2s[...] = pltpu.bitcast(w2_ref[...], jnp.uint32)
            d = dw_ref[...].astype(F32) * 0.5
            for c in range(NH):
                w = [jnp.broadcast_to(d[k:k + 1, c * 128:(c + 1) * 128], (8, 128)) for k in range(K)] + [None]

                def rec(w, path):
                    if len(path) == LV:
                        for j, v in enumerate(w):
                            if v is not None:
                                wt[c, pid[path], j] = v
                        return
                    e, o = w[0::2], w[1::2]
                    rec([a if b is None else a + b for a, b in zip(e, o)], path + (0,))
                    rec(e, path + (1,))
                    rec(o, path + (2,))
                rec(w, ())

        def glu(xv, c):
            w = pltpu.bitcast(w1s[c], BF)
            h = jnp.dot(xv, w, preferred_element_type=F32)
            return lambda r: h[r:r + 8, :128] * (jnp.tanh(h[r:r + 8, 128:]) + 1.0)

        def h_store(c, s, t, v):
            hb[c, t % TB // P, pl.ds(s * HS + t % P, 8), :] = v

        def h_load(c, t):
            return hb[c, t % TB // P, pl.ds(t % P, 8, stride=HS), :]

        def pw1(j, c, s0):
            xv = pltpu.bitcast(x_ref.bitcast(jnp.uint32)[s0:s0 + MS, pl.ds(j * P // 2, P // 2), :].reshape(MS * P // 2, D), BF)
            g = glu(xv, c)
            yield
            for s in range(MS):
                for q in range(P // 8):
                    h_store(c, s0 + s, j * P + q * 8, g(s * P + q * 8))
                yield

        def edge(ref, t0, ds):
            for c in range(NH):
                g = glu(ref[...].reshape(S * 16, D), c)
                for s in range(S):
                    src = s - ds
                    for q in range(2):
                        if 0 <= src < S and src // Q == s // Q:
                            v = g(src * 16 + q * 8)
                        else:
                            v = jnp.zeros((8, 128), F32)
                        h_store(c, s, t0 + q * 8, v)

        def pre(c, ms):
            @functools.cache
            def val(path, m):
                if not path:
                    return h_load(c, m - 15)
                p, b = path[:-1], path[-1]
                if b == 0:
                    return val(p, 2 * m + 1)
                return val(p, 2 * m + 2 * (b - 1)) - val(p, 2 * m + 1)
            for m in ms:
                for n, p in enumerate(paths[1:]):
                    sb[c, pid[p], m % RING] = val(p, m)
                    if n % 4 == 3:
                        yield

        def mac(c, m0, R=4):
            def leaf(path, init):
                n = 3 if path == (2,) * LV else 4
                if pid[path] == 0:
                    d = [h_load(c, 8 * (m0 + r) + 7 - 15) for r in range(R + n - 1)]
                else:
                    d = [sb[c, pid[path], (m0 + r) % RING] for r in range(R + n - 1)]
                w = [wt[c, pid[path], j] for j in range(n)]
                out = []
                for r in range(R):
                    a = None if init is None else init[r]
                    for j in range(n):
                        t = d[r + j] * w[j]
                        a = t if a is None else a + t
                    out.append(a)
                return out

            def rec(path, emit):
                n = R << (LV - len(path) - 1)
                if len(path) == LV - 1:
                    m1 = leaf(path + (0,), None)
                    yield
                    for b in (1, 2):
                        for r, v in enumerate(leaf(path + (b,), m1)):
                            emit(2 * r + b - 1, v)
                        yield
                    return
                m1 = [None] * n
                yield from rec(path + (0,), m1.__setitem__)
                for b in (1, 2):
                    yield from rec(path + (b,), lambda r, v, b=b: emit(2 * r + b - 1, v + m1[r]))

            def fin(r, y):
                t = (8 * m0 + r) % TB
                zz[r] = y * (jnp.tanh(y) + 1.0)
                if r ^ 1 in zz:
                    v = pltpu.pack_elementwise([zz[r & ~1], zz[r | 1]], packed_dtype=BF)
                    zb[c, t // P, pl.ds(t % P // 2, 8, stride=ZS), :] = v.astype(jnp.uint32)
            zz = {}
            yield from rec((), fin)

        def pw2(j, s0):
            z = pltpu.bitcast(jnp.concatenate([jnp.concatenate([zb[c, j, pl.ds(s * ZS + q * 8, 8), :] for s in range(s0, s0 + MS) for q in range(P // 16)], 0) for c in range(NH)], 1), BF)
            o = jnp.dot(z, pltpu.bitcast(w2s[...], BF), preferred_element_type=F32)
            yield
            for s in range(MS):
                o_ref[s0 + s, pl.ds(j * P, P), :] = o[s * P:(s + 1) * P].astype(o_ref.dtype)
                yield

        def mix(a, b):
            for _ in itertools.zip_longest(a, b):
                yield

        def step(i0):
            M = L // 8
            for js in grp:
              @pl.when(i < NS + 1 + js[0])
              def _():
               for j in js:
                g = i0 * NP + j
                ms = [m for m in range(4 * g - 3, 4 * g + 1) if 0 <= m < M + 3]
                domac = 0 <= g - 3 < L // P
                mm = []
                for s0 in range(0, S, MS):
                    if g >= NP:
                        mm.append(functools.partial(pw2, j, s0))
                    if g < L // P:
                        mm += [functools.partial(pw1, j, c, s0) for c in range(NH)]
                if od == 1: mm = mm[1:] + mm[:1]
                if od == 2: mm = [f for f in mm if f.func is pw1] + [f for f in mm if f.func is pw2]
                vp = itertools.chain(*[mix(itertools.chain(*[itertools.islice(mac(c, 4 * (g - 3) + r, R), 0, None, 4 // R) for r in range(0, 4, R)]) if domac else (), pre(c, ms)) for c in range(NH)])
                pass
                for n, f in enumerate(mm):
                    per = pp * (n + 1) // len(mm) - pp * n // len(mm)
                    gen = f()
                    next(gen)
                    for _ in itertools.islice(vp, 0):
                        pass
                    for _ in mix(itertools.islice(vp, per), gen):
                        pass
                for _ in vp:
                    pass

        @pl.when(i == 0)
        def _():
            weights()
            edge(xl_ref, -16, 1)
            step(0)

        @pl.when(jnp.logical_and(i > 0, i < NS))
        def _():
            step(1)

        @pl.when(i == NS)
        def _():
            edge(xf_ref, 0, -1)
            step(NS)

    xs = x.reshape(S, L, D)
    full = lambda a: pl.BlockSpec(a.shape, lambda i: (0, 0))
    hrows = HS * 8
    out = pl.pallas_call(
        kern, grid=(NS + 1,),
        in_specs=[pl.BlockSpec((S, TB, D), lambda i: (0, jnp.minimum(i, NS - 1), 0)),
                  pl.BlockSpec((S, 16, D), lambda i: (0, L // 16 - 1, 0)),
                  pl.BlockSpec((S, 16, D), lambda i: (0, 0, 0)),
                  full(w_pw1), full(dw), full(w_pw2)],
        out_specs=pl.BlockSpec((S, TB, D), lambda i: (0, jnp.maximum(i - 1, 0), 0)),
        out_shape=jax.ShapeDtypeStruct((S, L, D), x.dtype),
        scratch_shapes=[pltpu.VMEM((NH, D // 2, 256), jnp.uint32), pltpu.VMEM((D // 2, D), jnp.uint32), pltpu.VMEM((NH, 27, 4, 8, 128), F32),
                        pltpu.VMEM((NH, NP, hrows, 128), F32), pltpu.VMEM((NH, 27, RING, 8, 128), F32),
                        pltpu.VMEM((NH, NP, ZS * 8, 128), jnp.uint32)],
        compiler_params=pltpu.CompilerParams(dimension_semantics=("arbitrary",), vmem_limit_bytes=64 * 2**20, flags=flags),
    )(xs, xs, xs, w_pw1, dw, w_pw2)
    return out.reshape(B, T, D)
```

```python
import functools, itertools, jax, jax.numpy as jnp
import jax.experimental.pallas as pl
import jax.experimental.pallas.tpu as pltpu

F32 = jnp.float32
BF = jnp.bfloat16
S = 8
LV = 3


@jax.jit
def pallas_standalone__conformer_conv_module__speech_kernel(x, w_pw1, dw, w_pw2):
    NP, P, HS, ZS, MS, od, pp, sk, R, flags = 4, 80, 81, 41, 1, 2, 1.0, 1, 2, None
    sp = ((0, 48), (48, 32))
    B, T, D = x.shape
    K = dw.shape[0]
    Q = S // B
    L = T // Q
    TB = NP * P
    NS = -(-L // TB)
    G = L // P
    n8 = P // 8
    RING = TB // 8
    NH = D // 128
    paths = list(itertools.product(range(3), repeat=LV))
    pid = {p: i for i, p in enumerate(paths)}

    def kern(x_ref, xl_ref, xf_ref, w1_ref, dw_ref, w2_ref, o_ref, w1s, w2s, wt, hb, sb, zb):
        i = pl.program_id(0)

        def weights():
            for c in range(NH):
                w = jnp.concatenate([w1_ref[:, (e * NH + c) * 128:(e * NH + c + 1) * 128] for e in range(2)], 1)
                w1s[c] = pltpu.bitcast((w.astype(F32) * 0.5).astype(BF), jnp.uint32)
            w2s[...] = pltpu.bitcast(w2_ref[...], jnp.uint32)

        def taps():
            d = dw_ref[...].astype(F32) * 0.5
            for c in range(NH):
                w = [jnp.broadcast_to(d[k:k + 1, c * 128:(c + 1) * 128], (8, 128)) for k in range(K)] + [None]

                def rec(w, path):
                    if len(path) == LV:
                        for j, v in enumerate(w):
                            if v is not None:
                                wt[c, pid[path], j] = v
                        return
                    e, o = w[0::2], w[1::2]
                    rec([a if b is None else a + b for a, b in zip(e, o)], path + (0,))
                    rec(e, path + (1,))
                    rec(o, path + (2,))
                rec(w, ())

        def glu(xv, c):
            w = pltpu.bitcast(w1s[c], BF)
            h = jnp.dot(xv, w, preferred_element_type=F32)
            return lambda r: h[r:r + 8, :128] * (jnp.tanh(h[r:r + 8, 128:]) + 1.0)

        def h_store(c, s, t, v):
            hb[c, t % TB // P, pl.ds(s * HS + t % P, 8), :] = v

        def h_load(c, t):
            return hb[c, t % TB // P, pl.ds(t % P, 8, stride=HS), :]

        def pw1(j, c, s0, a, n):
            xv = pltpu.bitcast(x_ref.bitcast(jnp.uint32)[s0:s0 + MS, pl.ds((j * P + a) // 2, n // 2), :].reshape(n // 2, D), BF)
            g = glu(xv, c)
            yield
            for s in range(MS):
                for q in range(n // 8):
                    h_store(c, s0, j * P + a + q * 8, g(q * 8))
                yield

        def edge(ref, t0, ds):
            for c in range(NH):
                g = glu(ref[...].reshape(S * 16, D), c)
                for s in range(S):
                    src = s - ds
                    for q in range(2):
                        if 0 <= src < S and src // Q == s // Q:
                            v = g(src * 16 + q * 8)
                        else:
                            v = jnp.zeros((8, 128), F32)
                        h_store(c, s, t0 + q * 8, v)

        def pre(c, ms):
            @functools.cache
            def val(path, m):
                if not path:
                    return h_load(c, m - 15)
                p, b = path[:-1], path[-1]
                if b == 0:
                    return val(p, 2 * m + 1)
                return val(p, 2 * m + 2 * (b - 1)) - val(p, 2 * m + 1)
            for m in ms:
                for n, p in enumerate(paths[1:]):
                    sb[c, pid[p], m % RING] = val(p, m)
                    if n % 2 == 1:
                        yield

        def mac(c, m0, R=4):
            def leaf(path, init):
                n = 3 if path == (2,) * LV else 4
                if pid[path] == 0:
                    d = [h_load(c, 8 * (m0 + r) + 7 - 15) for r in range(R + n - 1)]
                else:
                    d = [sb[c, pid[path], (m0 + r) % RING] for r in range(R + n - 1)]
                w = [wt[c, pid[path], j] for j in range(n)]
                out = []
                for r in range(R):
                    a = None if init is None else init[r]
                    for j in range(n):
                        t = d[r + j] * w[j]
                        a = t if a is None else a + t
                    out.append(a)
                return out

            def rec(path, emit):
                n = R << (LV - len(path) - 1)
                if len(path) == LV - 1:
                    m1 = leaf(path + (0,), None)
                    yield
                    for b in (1, 2):
                        for r, v in enumerate(leaf(path + (b,), m1)):
                            emit(2 * r + b - 1, v)
                        yield
                    return
                m1 = [None] * n
                yield from rec(path + (0,), m1.__setitem__)
                for b in (1, 2):
                    yield from rec(path + (b,), lambda r, v, b=b: emit(2 * r + b - 1, v + m1[r]))

            def fin(r, y):
                t = (8 * m0 + r) % TB
                zz[r] = y * (jnp.tanh(y) + 1.0)
                if r ^ 1 in zz:
                    v = pltpu.pack_elementwise([zz[r & ~1], zz[r | 1]], packed_dtype=BF)
                    zb[c, t // P, pl.ds(t % P // 2, 8, stride=ZS), :] = v.astype(jnp.uint32)
            zz = {}
            yield from rec((), fin)

        def pw2(j, s0, a, n):
            z = pltpu.bitcast(jnp.concatenate([jnp.concatenate([zb[c, j, pl.ds(s * ZS + q * 8, 8), :] for s in range(s0, s0 + MS) for q in range(a // 16, (a + n) // 16)], 0) for c in range(NH)], 1), BF)
            o = jnp.dot(z, pltpu.bitcast(w2s[...], BF), preferred_element_type=F32)
            yield
            for s in range(MS):
                o_ref[s0 + s, pl.ds(j * P + a, n), :] = o.astype(o_ref.dtype)
                yield

        def mix(a, b):
            for _ in itertools.zip_longest(a, b):
                yield

        def step(i0):
            M = L // 8
            for j in range(NP):
              g = i0 * NP + j
              if g >= G + NP:
                  break

              @pl.when(i < NS + 1 + j)
              def _():
                if g == 1:
                    taps()
                if g == G - 1:
                    edge(xf_ref, L, -1)
                if True:
                    ms = [m for m in range(n8 * (g - 1) + 1, n8 * g + 1) if 0 <= m < M + 3]
                lo = lambda g: min(max(n8 * (g - 2) - 4, 0), M)
                m0s = range(lo(g), lo(g + 1), R)
                tot = int(NH * max(len(m0s) * 27, len(ms) * 13 // sk) * pp)
                mm = []
                for s0 in range(0, S, MS):
                    if g >= NP:
                        mm += [functools.partial(pw2, j, s0, *u) for u in (sp if m0s else [(0, P)])]
                    if g < L // P:
                        mm += [functools.partial(pw1, j, c, s0, *u) for c in range(NH) for u in (sp if m0s else [(0, P)])]
                if od == 1: mm = mm[1:] + mm[:1]
                if od == 2: mm = [f for f in mm if f.func is pw1] + [f for f in mm if f.func is pw2]
                vp = itertools.chain(*[mix(itertools.chain(*[mac(c, m, R) for m in m0s]), itertools.islice(pre(c, ms), 0, None, sk)) for c in range(NH)])
                pass
                for n, f in enumerate(mm):
                    per = tot * (n + 1) // len(mm) - tot * n // len(mm)
                    gen = f()
                    next(gen)
                    for _ in itertools.islice(vp, 0):
                        pass
                    for _ in mix(itertools.islice(vp, per), gen):
                        pass
                for _ in vp:
                    pass

        @pl.when(i == 0)
        def _():
            weights()
            edge(xl_ref, -16, 1)
            step(0)

        @pl.when(jnp.logical_and(i > 0, i < G // NP))
        def _():
            step(1)

        for e in range(G // NP, NS + 1):
            pl.when(i == e)(functools.partial(step, e))

    xs = x.reshape(S, L, D)
    full = lambda a: pl.BlockSpec(a.shape, lambda i: (0, 0))
    hrows = HS * 8
    out = pl.pallas_call(
        kern, grid=(NS + 1,),
        in_specs=[pl.BlockSpec((S, TB, D), lambda i: (0, jnp.minimum(i, NS - 1), 0)),
                  pl.BlockSpec((S, 16, D), lambda i: (0, L // 16 - 1, 0)),
                  pl.BlockSpec((S, 16, D), lambda i: (0, 0, 0)),
                  full(w_pw1), full(dw), full(w_pw2)],
        out_specs=pl.BlockSpec((S, TB, D), lambda i: (0, jnp.maximum(i - 1, 0), 0)),
        out_shape=jax.ShapeDtypeStruct((S, L, D), x.dtype),
        scratch_shapes=[pltpu.VMEM((NH, D // 2, 256), jnp.uint32), pltpu.VMEM((D // 2, D), jnp.uint32), pltpu.VMEM((NH, 27, 4, 8, 128), F32),
                        pltpu.VMEM((NH, NP, hrows, 128), F32), pltpu.VMEM((NH, 27, RING, 8, 128), F32),
                        pltpu.VMEM((NH, NP, ZS * 8, 128), jnp.uint32)],
        compiler_params=pltpu.CompilerParams(dimension_semantics=("arbitrary",), vmem_limit_bytes=64 * 2**20, flags=flags),
    )(xs, xs, xs, w_pw1, dw, w_pw2)
    return out.reshape(B, T, D)
```

```python
import functools, itertools, jax, jax.numpy as jnp
import jax.experimental.pallas as pl
import jax.experimental.pallas.tpu as pltpu

F32 = jnp.float32
BF = jnp.bfloat16
S = 8
LV = 3


@jax.jit
def pallas_standalone__conformer_conv_module__speech_kernel(x, w_pw1, dw, w_pw2):
    NP, P, HS, ZS, MS, od, pp, sk, R, flags = 4, 80, 81, 41, 1, 2, 1.0, 1, 2, None
    sp = ((0, 48), (48, 32))
    B, T, D = x.shape
    K = dw.shape[0]
    Q = S // B
    L = T // Q
    TB = NP * P
    NS = -(-L // TB)
    G = L // P
    n8 = P // 8
    RING = TB // 8
    NH = D // 128
    paths = list(itertools.product(range(3), repeat=LV))
    pid = {p: i for i, p in enumerate(paths)}

    def kern(x_hbm, xl_ref, xf_ref, w1_ref, dw_ref, w2_ref, o_hbm, xb, o_ref, xsem, osem, sm, w1s, w2s, wt, hb, sb, zb):
        x_ref = xb

        def xcp(g, j):
            return pltpu.make_async_copy(x_hbm.at[:, pl.ds(pl.multiple_of(g * P, P), P), :], xb.at[:, pl.ds(j * P, P), :], xsem.at[j])

        def ocp(g, j):
            return pltpu.make_async_copy(o_ref.at[:, pl.ds(j * P, P), :], o_hbm.at[:, pl.ds(pl.multiple_of(g * P, P), P), :], osem.at[j])

        def weights():
            for c in range(NH):
                w = jnp.concatenate([w1_ref[:, (e * NH + c) * 128:(e * NH + c + 1) * 128] for e in range(2)], 1)
                w1s[c] = pltpu.bitcast((w.astype(F32) * 0.5).astype(BF), jnp.uint32)
            w2s[...] = pltpu.bitcast(w2_ref[...], jnp.uint32)

        def taps():
            d = dw_ref[...].astype(F32) * 0.5
            for c in range(NH):
                w = [jnp.broadcast_to(d[k:k + 1, c * 128:(c + 1) * 128], (8, 128)) for k in range(K)] + [None]

                def rec(w, path):
                    if len(path) == LV:
                        for j, v in enumerate(w):
                            if v is not None:
                                wt[c, pid[path], j] = v
                        return
                    e, o = w[0::2], w[1::2]
                    rec([a if b is None else a + b for a, b in zip(e, o)], path + (0,))
                    rec(e, path + (1,))
                    rec(o, path + (2,))
                rec(w, ())

        def glu(xv, c):
            w = pltpu.bitcast(w1s[c], BF)
            h = jnp.dot(xv, w, preferred_element_type=F32)
            return lambda r: h[r:r + 8, :128] * (jnp.tanh(h[r:r + 8, 128:]) + 1.0)

        def h_store(c, s, t, v):
            hb[c, t % TB // P, pl.ds(s * HS + t % P, 8), :] = v

        def h_load(c, t):
            return hb[c, t % TB // P, pl.ds(t % P, 8, stride=HS), :]

        def pw1(j, c, s0, a, n):
            xv = pltpu.bitcast(x_ref.bitcast(jnp.uint32)[s0:s0 + MS, pl.ds((j * P + a) // 2, n // 2), :].reshape(n // 2, D), BF)
            g = glu(xv, c)
            yield
            for s in range(MS):
                for q in range(n // 8):
                    h_store(c, s0, j * P + a + q * 8, g(q * 8))
                yield

        def edge(ref, t0, ds):
            for c in range(NH):
                g = glu(ref[...].reshape(S * 16, D), c)
                for s in range(S):
                    src = s - ds
                    for q in range(2):
                        if 0 <= src < S and src // Q == s // Q:
                            v = g(src * 16 + q * 8)
                        else:
                            v = jnp.zeros((8, 128), F32)
                        h_store(c, s, t0 + q * 8, v)

        def pre(c, ms):
            @functools.cache
            def val(path, m):
                if not path:
                    return h_load(c, m - 15)
                p, b = path[:-1], path[-1]
                if b == 0:
                    return val(p, 2 * m + 1)
                return val(p, 2 * m + 2 * (b - 1)) - val(p, 2 * m + 1)
            for m in ms:
                for n, p in enumerate(paths[1:]):
                    sb[c, pid[p], m % RING] = val(p, m)
                    if n % 2 == 1:
                        yield

        def mac(c, m0, R=4):
            def leaf(path, init):
                n = 3 if path == (2,) * LV else 4
                if pid[path] == 0:
                    d = [h_load(c, 8 * (m0 + r) + 7 - 15) for r in range(R + n - 1)]
                else:
                    d = [sb[c, pid[path], (m0 + r) % RING] for r in range(R + n - 1)]
                w = [wt[c, pid[path], j] for j in range(n)]
                out = []
                for r in range(R):
                    a = None if init is None else init[r]
                    for j in range(n):
                        t = d[r + j] * w[j]
                        a = t if a is None else a + t
                    out.append(a)
                return out

            def rec(path, emit):
                n = R << (LV - len(path) - 1)
                if len(path) == LV - 1:
                    m1 = leaf(path + (0,), None)
                    yield
                    for b in (1, 2):
                        for r, v in enumerate(leaf(path + (b,), m1)):
                            emit(2 * r + b - 1, v)
                        yield
                    return
                m1 = [None] * n
                yield from rec(path + (0,), m1.__setitem__)
                for b in (1, 2):
                    yield from rec(path + (b,), lambda r, v, b=b: emit(2 * r + b - 1, v + m1[r]))

            def fin(r, y):
                t = (8 * m0 + r) % TB
                zz[r] = y * (jnp.tanh(y) + 1.0)
                if r ^ 1 in zz:
                    v = pltpu.pack_elementwise([zz[r & ~1], zz[r | 1]], packed_dtype=BF)
                    zb[c, t // P, pl.ds(t % P // 2, 8, stride=ZS), :] = v.astype(jnp.uint32)
            zz = {}
            yield from rec((), fin)

        def pw2(j, s0, a, n):
            z = pltpu.bitcast(jnp.concatenate([jnp.concatenate([zb[c, j, pl.ds(s * ZS + q * 8, 8), :] for s in range(s0, s0 + MS) for q in range(a // 16, (a + n) // 16)], 0) for c in range(NH)], 1), BF)
            o = jnp.dot(z, pltpu.bitcast(w2s[...], BF), preferred_element_type=F32)
            yield
            for s in range(MS):
                o_ref[s0 + s, pl.ds(j * P + a, n), :] = o.astype(o_ref.dtype)
                yield

        def mix(a, b):
            for _ in itertools.zip_longest(a, b):
                yield

        def step(i0, i):
            M = L // 8
            for j in range(NP):
              g = i0 * NP + j
              if g >= G + NP:
                  break

              gd = i * NP + j
              if g + 2 < G:
                  xcp(gd + 2, (j + 2) % NP).start()
              if g < G:
                  xcp(gd, j).wait()
              if i0 == 1:
                  pl.when(i > 1)(lambda: ocp(0, j).wait())
              elif i0 > 1:
                  ocp(0, j).wait()

              @pl.when(sm[0] < 1 + g)
              def _():
                if g == 1:
                    taps()
                if g == G - 1:
                    edge(xf_ref, L, -1)
                if True:
                    ms = [m for m in range(n8 * (g - 1) + 1, n8 * g + 1) if 0 <= m < M + 3]
                lo = lambda g: min(max(n8 * (g - 2) - 4, 0), M)
                m0s = range(lo(g), lo(g + 1), R)
                tot = int(NH * max(len(m0s) * 27, len(ms) * 13 // sk) * pp)
                mm = []
                for s0 in range(0, S, MS):
                    if g >= NP:
                        mm += [functools.partial(pw2, j, s0, *u) for u in sp]
                    if g < L // P:
                        mm += [functools.partial(pw1, j, c, s0, *u) for c in range(NH) for u in sp]
                if od == 1: mm = mm[1:] + mm[:1]
                if od == 2: mm = [f for f in mm if f.func is pw1] + [f for f in mm if f.func is pw2]
                vp = itertools.chain(*[mix(itertools.chain(*[mac(c, m, R) for m in m0s]), itertools.islice(pre(c, ms), 0, None, sk)) for c in range(NH)])
                pass
                for n, f in enumerate(mm):
                    per = tot * (n + 1) // len(mm) - tot * n // len(mm)
                    gen = f()
                    next(gen)
                    for _ in itertools.islice(vp, 0):
                        pass
                    for _ in mix(itertools.islice(vp, per), gen):
                        pass
                for _ in vp:
                    pass

              if g >= NP:
                  ocp(gd - NP, j).start()

        sm[0] = 0
        i0 = 0
        xcp(0, 0).start()
        xcp(1, 1).start()
        weights()
        edge(xl_ref, -16, 1)
        step(0, i0)
        pl.loop(1, G // NP)(functools.partial(step, 1))
        for e in range(G // NP, NS + 1):
            step(e, i0 + e)
        for j in range(NP):
            ocp(0, j).wait()

    xs = x.reshape(S, L, D)
    full = lambda a: pl.BlockSpec(a.shape, lambda i: (0, 0))
    hrows = HS * 8
    out = pl.pallas_call(
        kern, grid=(1,),
        in_specs=[pl.BlockSpec(memory_space=pl.ANY),
                  pl.BlockSpec((S, 16, D), lambda i: (0, L // 16 - 1, 0)),
                  pl.BlockSpec((S, 16, D), lambda i: (0, 0, 0)),
                  full(w_pw1), full(dw), full(w_pw2)],
        out_specs=pl.BlockSpec(memory_space=pl.ANY),
        out_shape=jax.ShapeDtypeStruct((S, L, D), x.dtype),
        scratch_shapes=[pltpu.VMEM((S, TB, D), BF), pltpu.VMEM((S, TB, D), BF),
                        pltpu.SemaphoreType.DMA((NP,)), pltpu.SemaphoreType.DMA((NP,)), pltpu.SMEM((1,), jnp.int32),
                        pltpu.VMEM((NH, D // 2, 256), jnp.uint32), pltpu.VMEM((D // 2, D), jnp.uint32), pltpu.VMEM((NH, 27, 4, 8, 128), F32),
                        pltpu.VMEM((NH, NP, hrows, 128), F32), pltpu.VMEM((NH, 27, RING, 8, 128), F32),
                        pltpu.VMEM((NH, NP, ZS * 8, 128), jnp.uint32)],
        compiler_params=pltpu.CompilerParams(dimension_semantics=("arbitrary",), vmem_limit_bytes=64 * 2**20, flags=flags),
    )(xs, xs, xs, w_pw1, dw, w_pw2)
    return out.reshape(B, T, D)
```

```python
import functools, itertools, jax, jax.numpy as jnp
import jax.experimental.pallas as pl
import jax.experimental.pallas.tpu as pltpu

F32 = jnp.float32
BF = jnp.bfloat16
S = 8
LV = 3


@jax.jit
def pallas_standalone__conformer_conv_module__speech_kernel(x, w_pw1, dw, w_pw2):
    NP, P, HS, MS, od, pp, sk, R, flags = 4, 80, 81, 1, 2, 1.0, 1, 2, None
    sp = ((0, 48), (48, 32))
    B, T, D = x.shape
    K = dw.shape[0]
    Q = S // B
    L = T // Q
    TB = NP * P
    NS = -(-L // TB)
    G = L // P
    n8 = P // 8
    RING = TB // 8
    NH = D // 128
    paths = list(itertools.product(range(3), repeat=LV))
    pid = {p: i for i, p in enumerate(paths)}

    def kern(x_hbm, xl_ref, xf_ref, w1_ref, dw_ref, w2_ref, o_hbm, xb, o_ref, xsem, osem, sm, w1s, w2s, wt, hb, sb, zb):
        x_ref = xb

        def xcp(g, j):
            return pltpu.make_async_copy(x_hbm.at[:, pl.ds(pl.multiple_of(g * P, P), P), :], xb.at[:, pl.ds(j * P, P), :], xsem.at[j])

        def ocp(g, j):
            return pltpu.make_async_copy(o_ref.at[:, pl.ds(j * P, P), :], o_hbm.at[:, pl.ds(pl.multiple_of(g * P, P), P), :], osem.at[j])

        def weights():
            for c in range(NH):
                w = jnp.concatenate([w1_ref[:, (e * NH + c) * 128:(e * NH + c + 1) * 128] for e in range(2)], 1)
                w1s[c] = pltpu.bitcast((w.astype(F32) * 0.5).astype(BF), jnp.uint32)
            w2s[...] = pltpu.bitcast(w2_ref[...], jnp.uint32)

        def taps():
            d = dw_ref[...].astype(F32) * 0.5
            for c in range(NH):
                w = [jnp.broadcast_to(d[k:k + 1, c * 128:(c + 1) * 128], (8, 128)) for k in range(K)] + [None]

                def rec(w, path):
                    if len(path) == LV:
                        for j, v in enumerate(w):
                            if v is not None:
                                wt[c, pid[path], j] = v
                        return
                    e, o = w[0::2], w[1::2]
                    rec([a if b is None else a + b for a, b in zip(e, o)], path + (0,))
                    rec(e, path + (1,))
                    rec(o, path + (2,))
                rec(w, ())

        def glu(xv, c):
            w = pltpu.bitcast(w1s[c], BF)
            h = jnp.dot(xv, w, preferred_element_type=F32)
            return lambda r: h[r:r + 8, :128] * (jnp.tanh(h[r:r + 8, 128:]) + 1.0)

        def h_store(c, s, t, v):
            hb[c, t % TB // P, pl.ds(s * HS + t % P, 8), :] = v

        def h_load(c, t):
            return hb[c, t % TB // P, pl.ds(t % P, 8, stride=HS), :]

        def pw1(j, c, s0, a, n):
            xv = x_ref[s0, pl.ds(j * P + a, n), :]
            g = glu(xv, c)
            yield
            for s in range(MS):
                for q in range(n // 8):
                    h_store(c, s0, j * P + a + q * 8, g(q * 8))
                yield

        def edge(ref, t0, ds):
            for c in range(NH):
                g = glu(ref[...].reshape(S * 16, D), c)
                for s in range(S):
                    src = s - ds
                    for q in range(2):
                        if 0 <= src < S and src // Q == s // Q:
                            v = g(src * 16 + q * 8)
                        else:
                            v = jnp.zeros((8, 128), F32)
                        h_store(c, s, t0 + q * 8, v)

        def pre(c, ms):
            @functools.cache
            def val(path, m):
                if not path:
                    return h_load(c, m - 15)
                p, b = path[:-1], path[-1]
                if b == 0:
                    return val(p, 2 * m + 1)
                return val(p, 2 * m + 2 * (b - 1)) - val(p, 2 * m + 1)
            for m in ms:
                for n, p in enumerate(paths[1:]):
                    sb[c, pid[p], m % RING] = val(p, m)
                    if n % 2 == 1:
                        yield

        def mac(c, m0, R=4):
            def leaf(path, init):
                n = 3 if path == (2,) * LV else 4
                if pid[path] == 0:
                    d = [h_load(c, 8 * (m0 + r) + 7 - 15) for r in range(R + n - 1)]
                else:
                    d = [sb[c, pid[path], (m0 + r) % RING] for r in range(R + n - 1)]
                w = [wt[c, pid[path], j] for j in range(n)]
                out = []
                for r in range(R):
                    a = None if init is None else init[r]
                    for j in range(n):
                        t = d[r + j] * w[j]
                        a = t if a is None else a + t
                    out.append(a)
                return out

            def rec(path, emit):
                n = R << (LV - len(path) - 1)
                if len(path) == LV - 1:
                    m1 = leaf(path + (0,), None)
                    yield
                    for b in (1, 2):
                        for r, v in enumerate(leaf(path + (b,), m1)):
                            emit(2 * r + b - 1, v)
                        yield
                    return
                m1 = [None] * n
                yield from rec(path + (0,), m1.__setitem__)
                for b in (1, 2):
                    yield from rec(path + (b,), lambda r, v, b=b: emit(2 * r + b - 1, v + m1[r]))

            def fin(r, y):
                t = (8 * m0 + r) % TB
                zb[c, t // P, pl.ds(t % P, 8, stride=HS), :] = y * (jnp.tanh(y) + 1.0)
            yield from rec((), fin)

        def pw2(j, s0, a, n):
            z = jnp.concatenate([jnp.concatenate([zb[c, j, pl.ds(s0 * HS + q * 8, 8), :] for q in range(a // 8, (a + n) // 8)], 0) for c in range(NH)], 1).astype(BF)
            o = jnp.dot(z, pltpu.bitcast(w2s[...], BF), preferred_element_type=F32)
            yield
            for s in range(MS):
                o_ref[s0 + s, pl.ds(j * P + a, n), :] = o.astype(o_ref.dtype)
                yield

        def mix(a, b):
            for _ in itertools.zip_longest(a, b):
                yield

        def step(i0, i):
            M = L // 8
            for j in range(NP):
              g = i0 * NP + j
              if g >= G + NP:
                  break

              gd = i * NP + j
              if g + 2 < G:
                  xcp(gd + 2, (j + 2) % NP).start()
              if g < G:
                  xcp(gd, j).wait()
              if i0 == 1:
                  pl.when(i > 1)(lambda: ocp(0, j).wait())
              elif i0 > 1:
                  ocp(0, j).wait()

              @pl.when(sm[0] < 1 + g)
              def _():
                if g == 1:
                    taps()
                if g == G - 1:
                    edge(xf_ref, L, -1)
                if True:
                    ms = [m for m in range(n8 * (g - 1) + 1, n8 * g + 1) if 0 <= m < M + 3]
                lo = lambda g: min(max(n8 * (g - 2) - 4, 0), M)
                m0s = range(lo(g), lo(g + 1), R)
                tot = int(NH * max(len(m0s) * 27, len(ms) * 13 // sk) * pp)
                mm = []
                for s0 in range(0, S, MS):
                    if g >= NP:
                        mm += [functools.partial(pw2, j, s0, *u) for u in sp]
                    if g < L // P:
                        mm += [functools.partial(pw1, j, c, s0, *u) for c in range(NH) for u in sp]
                if od == 1: mm = mm[1:] + mm[:1]
                if od == 2: mm = [f for f in mm if f.func is pw1] + [f for f in mm if f.func is pw2]
                vp = itertools.chain(*[mix(itertools.chain(*[mac(c, m, R) for m in m0s]), itertools.islice(pre(c, ms), 0, None, sk)) for c in range(NH)])
                pass
                for n, f in enumerate(mm):
                    per = tot * (n + 1) // len(mm) - tot * n // len(mm)
                    gen = f()
                    next(gen)
                    for _ in itertools.islice(vp, 0):
                        pass
                    for _ in mix(itertools.islice(vp, per), gen):
                        pass
                for _ in vp:
                    pass

              if g >= NP:
                  ocp(gd - NP, j).start()

        sm[0] = 0
        i0 = 0
        xcp(0, 0).start()
        xcp(1, 1).start()
        weights()
        edge(xl_ref, -16, 1)
        step(0, i0)
        pl.loop(1, G // NP)(functools.partial(step, 1))
        for e in range(G // NP, NS + 1):
            step(e, i0 + e)
        for j in range(NP):
            ocp(0, j).wait()

    xs = x.reshape(S, L, D)
    full = lambda a: pl.BlockSpec(a.shape, lambda i: (0, 0))
    hrows = HS * 8
    out = pl.pallas_call(
        kern, grid=(1,),
        in_specs=[pl.BlockSpec(memory_space=pl.ANY),
                  pl.BlockSpec((S, 16, D), lambda i: (0, L // 16 - 1, 0)),
                  pl.BlockSpec((S, 16, D), lambda i: (0, 0, 0)),
                  full(w_pw1), full(dw), full(w_pw2)],
        out_specs=pl.BlockSpec(memory_space=pl.ANY),
        out_shape=jax.ShapeDtypeStruct((S, L, D), x.dtype),
        scratch_shapes=[pltpu.VMEM((S, TB, D), BF), pltpu.VMEM((S, TB, D), BF),
                        pltpu.SemaphoreType.DMA((NP,)), pltpu.SemaphoreType.DMA((NP,)), pltpu.SMEM((1,), jnp.int32),
                        pltpu.VMEM((NH, D // 2, 256), jnp.uint32), pltpu.VMEM((D // 2, D), jnp.uint32), pltpu.VMEM((NH, 27, 4, 8, 128), F32),
                        pltpu.VMEM((NH, NP, hrows, 128), F32), pltpu.VMEM((NH, 27, RING, 8, 128), F32),
                        pltpu.VMEM((NH, NP, hrows, 128), F32)],
        compiler_params=pltpu.CompilerParams(dimension_semantics=("arbitrary",), vmem_limit_bytes=64 * 2**20, flags=flags),
    )(xs, xs, xs, w_pw1, dw, w_pw2)
    return out.reshape(B, T, D)
```
